```python
import os as _os
_os.environ.setdefault('JAX_PLATFORMS', 'cpu')
import jax
import jax.numpy as jnp

def _softmax(x, axis=-1):
    return jax.nn.softmax(x, axis=axis)

def _gelu(x):
    return jax.nn.gelu(x, approximate=True)

def _silu(x):
    return jax.nn.silu(x)

def _sigmoid(x):
    return jax.nn.sigmoid(x)

def _layernorm(x, axis=-1, eps=1e-05):
    m = jnp.mean(x, axis=axis, keepdims=True)
    v = jnp.var(x, axis=axis, keepdims=True)
    return (x - m) / jnp.sqrt(v + eps)

def _scatter_add(tgt, idx, src, axis=0):
    return tgt.at[idx].add(src)

def _segment_sum(src, seg, n):
    return jax.ops.segment_sum(src, seg, n)

class _Rng:

    def __init__(self, key):
        self._k = key

    def _next(self):
        self._k, sub = jax.random.split(self._k)
        return sub

    def normal(self, shape):
        return jax.random.normal(self._next(), shape, dtype=jnp.bfloat16)

    def randint(self, lo, hi, shape):
        return jax.random.randint(self._next(), shape, lo, hi, dtype=jnp.int32)

    def uniform(self, shape, lo=0.0, hi=1.0):
        return jax.random.uniform(self._next(), shape, jnp.bfloat16, lo, hi)

    def permutation(self, n):
        return jax.random.permutation(self._next(), n)
kernel_name = 'sequential_preLN__memory_aug_recurrent_mem_tr__swiglu_ffn__prompt'

def setup_inputs():
    _rng = _Rng(jax.random.key(int.from_bytes(__import__("os").urandom(4), "little")))
    _w = lambda a: (lambda t: t.astype(jnp.bfloat16) if jnp.issubdtype(t.dtype, jnp.floating) else t)(jnp.asarray(a))

    def _A_setup():
        B, S, Dm = (1, 2048, 640)
        H, Dh = (32, 192)
        M, seg = (8, 32)
        seg = min(seg, S)
        S = S // seg * seg
        return {'x': _w((lambda *s: _rng.normal(s) * 0.05)(B, S, Dm)), 'mem0': _w((lambda *s: _rng.normal(s) * 0.1)(B, M, Dm)), 'Wq': _w((lambda *s: _rng.normal(s) * 1.6)(Dm, H, Dh) * Dm ** (-0.5)), 'Wk': _w((lambda *s: _rng.normal(s) * 1.6)(Dm, H, Dh) * Dm ** (-0.5)), 'Wv': _w((lambda *s: _rng.normal(s) * 0.1)(Dm, H, Dh) * Dm ** (-0.5)), 'Wo': _w((lambda *s: _rng.normal(s) * 0.1)(H, Dh, Dm) * (H * Dh) ** (-0.5)), 'seg_len': seg}
    _A_in = _A_setup()

    def _B_setup():
        B, S, D, F = (1, 2048, 640, 1536)
        return {'x': _w((lambda *s: _rng.normal(s) * 0.05)(B, S, D)), 'w_gate': _w((lambda *s: _rng.normal(s) * 0.05)(D, F)), 'w_up': _w((lambda *s: _rng.normal(s) * 0.05)(D, F)), 'w_down': _w((lambda *s: _rng.normal(s) * 0.05)(F, D))}
    _B_in = _B_setup()
    return {'A_x': _A_in['x'], 'A_mem0': _A_in['mem0'], 'A_Wq': _A_in['Wq'], 'A_Wk': _A_in['Wk'], 'A_Wv': _A_in['Wv'], 'A_Wo': _A_in['Wo'], 'A_seg_len': _A_in['seg_len'], 'B_x': _B_in['x'], 'B_w_gate': _B_in['w_gate'], 'B_w_up': _B_in['w_up'], 'B_w_down': _B_in['w_down']}

def reference(A_x, A_mem0, A_Wq, A_Wk, A_Wv, A_Wo, A_seg_len, B_x, B_w_gate, B_w_up, B_w_down):

    def _A_ref(x, mem0, Wq, Wk, Wv, Wo, seg_len):
        B, S, Dm = x.shape
        H, Dh = (Wq.shape[1], Wq.shape[2])
        M = mem0.shape[1]
        scale = Dh ** (-0.5)
        n_seg = S // seg_len
        L = M + seg_len
        idx = jnp.arange(L)
        mask = (idx[:, None] < M) | (idx[:, None] >= idx[None, :])
        mem = mem0
        outs = []
        for s in range(n_seg):
            xs = x[:, s * seg_len:(s + 1) * seg_len, :].copy()
            h = jnp.concatenate([mem, xs], axis=1)
            q = jnp.einsum('btd,dhe->bhte', h, Wq)
            k = jnp.einsum('btd,dhe->bhte', h, Wk)
            v = jnp.einsum('btd,dhe->bhte', h, Wv)
            scores = jnp.einsum('bhqe,bhke->bhqk', q, k) * scale
            scores = jnp.where(mask[None, None], scores, -1000000000.0)
            p = _softmax(scores, axis=-1)
            o = jnp.einsum('bhqk,bhke->bhqe', p, v)
            o = jnp.einsum('bhte,hed->btd', o, Wo)
            mem = o[:, :M, :].copy()
            outs.append(o[:, M:, :])
        return jnp.concatenate(outs, axis=1)

    def _B_ref(x, w_gate, w_up, w_down):
        g = _silu(x @ w_gate)
        u = x @ w_up
        return g * u @ w_down
    x = A_x
    h = x + _A_ref(_layernorm(x, axis=-1), A_mem0, A_Wq, A_Wk, A_Wv, A_Wo, A_seg_len)
    h2 = h + _B_ref(_layernorm(h, axis=-1), B_w_gate, B_w_up, B_w_down)
    return h2
```

```python
import functools
import jax
import jax.numpy as jnp
import numpy as np
from jax.experimental import pallas as pl
from jax.experimental.pallas import tpu as pltpu

F32 = jnp.float32
BF16 = jnp.bfloat16
NT = (((1,), (1,)), ((), ()))


def _ln(x):
    m = jnp.mean(x, axis=-1, keepdims=True)
    d = x - m
    v = jnp.mean(d * d, axis=-1, keepdims=True)
    return d * jax.lax.rsqrt(v + 1e-5)


def _dot(a, b):
    return jnp.dot(a, b, preferred_element_type=F32)


def make_kernel(S, D, H, Dh, M, SEG, F, NA, lag_s=1, lag_pv=2, lag_o=5, ahead=3, nsteps=None, tg=0, unroll=1, tail='SOOVOVOO'):
    NP = H // 2
    PW = 2 * Dh
    L = M + SEG
    NSEG = S // SEG
    PRE = 8
    scale = float(Dh) ** -0.5
    AHEAD = ahead

    def order(full):
        ops = []
        if full:
            for t in range(NP):
                if t == tg:
                    ops.append(('F', 0))
                ops.append(('P', t))
                for op, lag in (('S', lag_s), ('V', lag_pv), ('O', lag_o)):
                    if t - lag >= 0:
                        ops.append((op, t - lag))
            rest = {op: [p for p in range(NP - lag, NP)] for op, lag in (('S', lag_s), ('V', lag_pv), ('O', lag_o))}
            for op in tail:
                ops.append((op, rest[op].pop(0)))
            assert not any(rest.values())
        else:
            for t in range(NP + 5):
                for op, lag in (('P', 0), ('S', 0), ('V', 3), ('O', 5)):
                    if 0 <= t - lag < NP:
                        ops.append((op, t - lag))
        return ops

    def kernel(x_hbm, mem0_ref, wq_hbm, wk_hbm, wv_hbm, wo_hbm, wg_hbm, wu_hbm, wd_hbm,
               o_hbm,
               x_v, o_v, stage, wqkv, wo_v, wg_v, wu_v, wd_v, lhs0, pbuf, h_v, hn_v, a_v,
               sem_w, sem_x, sem_f, sem_o):

        def w_copies(p):
            r = pl.ds(pl.multiple_of(p * PW, PW), PW)
            return [
                pltpu.make_async_copy(wk_hbm.at[r, :], stage.at[p, 0], sem_w.at[p, 0]),
                pltpu.make_async_copy(wv_hbm.at[r, :], stage.at[p, 1], sem_w.at[p, 1]),
                pltpu.make_async_copy(wq_hbm.at[r, :], stage.at[p, 2], sem_w.at[p, 2]),
                pltpu.make_async_copy(wo_hbm.at[r, :], wo_v.at[p], sem_w.at[p, 3]),
            ]

        x_copy = pltpu.make_async_copy(x_hbm, x_v, sem_x.at[0])
        f_copies = [
            pltpu.make_async_copy(wg_hbm, wg_v, sem_f.at[0]),
            pltpu.make_async_copy(wu_hbm, wu_v, sem_f.at[1]),
            pltpu.make_async_copy(wd_hbm, wd_v, sem_f.at[2]),
        ]
        x_copy.start()
        for p in range(AHEAD):
            for c in w_copies(p):
                c.start()

        row = jax.lax.broadcasted_iota(jnp.int32, (L, 2 * L), 0)
        col = jax.lax.broadcasted_iota(jnp.int32, (L, 2 * L), 1)
        first = col < L
        key = jnp.where(first, col, col - L)
        visible = (row < M) | (row >= key)
        lane = jax.lax.broadcasted_iota(jnp.int32, (L, PW), 1)
        lo_half = lane < Dh

        def blockdiag(t):
            a = jnp.where(lo_half, t, 0.0)
            b = jnp.where(lo_half, 0.0, t)
            return jnp.concatenate([a, b], axis=0).astype(BF16)

        def scores(q, kbd):
            s = jax.lax.dot_general(q, kbd, NT, preferred_element_type=F32)
            s = jnp.where(visible, s * scale, -1e9)
            m0 = jnp.max(jnp.where(first, s, -jnp.inf), axis=-1, keepdims=True)
            m1 = jnp.max(jnp.where(first, -jnp.inf, s), axis=-1, keepdims=True)
            e = jnp.exp(s - jnp.where(first, m0, m1))
            l0 = jnp.sum(jnp.where(first, e, 0.0), axis=-1, keepdims=True)
            l1 = jnp.sum(jnp.where(first, 0.0, e), axis=-1, keepdims=True)
            return e * jnp.where(first, 1.0 / l0, 1.0 / l1)

        def rows(s):
            return pl.ds(pl.multiple_of(s * SEG, SEG), SEG)

        def ffn_up():
            hn = hn_v[...]
            g = _dot(hn, wg_v[...])
            u = _dot(hn, wu_v[...])
            a_v[...] = (g * jax.nn.sigmoid(g) * u).astype(BF16)

        def ffn_down(s):
            y = _dot(a_v[...], wd_v[...])
            o_v[rows(s), :] = (h_v[...] + y).astype(o_v.dtype)

        def finish(xs, acc):
            hres = xs + acc[M:]
            hn_v[...] = _ln(hres).astype(BF16)
            return hres

        def attend(proj, extra=None):
            qkv, pr, ov = {}, {}, {}
            acc = [None]

            def do(op, p):
                if op == 'P':
                    kbd = blockdiag(proj(p, 0))
                    vbd = blockdiag(proj(p, 1))
                    qkv[p] = (proj(p, 2), kbd, vbd)
                elif op == 'S':
                    pr[p] = scores(qkv[p][0], qkv[p][1])
                elif op == 'V':
                    ov[p] = _dot(pr[p], qkv[p][2])
                elif op == 'O':
                    c = _dot(ov[p], wo_v[p])
                    acc[0] = c if acc[0] is None else acc[0] + c
                else:
                    extra()

            for op, p in order(extra is not None):
                do(op, p)
            return acc[0]

        def step(s, mem, pre):
            xs = x_v[rows(s), :].astype(F32)
            nt = SEG - PRE if pre else SEG
            h = jnp.concatenate([mem, _ln(xs[:nt])], axis=0)
            prow = pl.ds(pl.multiple_of(L + (s - 1) * PRE, PRE), PRE)

            def proj(p, j):
                t = _dot(h, wqkv[p, j])
                if pre:
                    t = jnp.concatenate([t, pbuf[p, j, prow, :]], axis=0)
                return t

            acc = attend(proj, ffn_up)
            hres = finish(x_v[rows(s), :].astype(F32), acc)
            ffn_down(s - 1)
            h_v[...] = hres
            return acc[:M]

        x_copy.wait()
        lhs0[0:M, :] = mem0_ref[...].astype(F32)
        lhs0[M:L, :] = _ln(x_v[0:SEG, :].astype(F32))
        for s in range(1, NA + 1):
            xs = x_v[s * SEG + SEG - 16:(s + 1) * SEG, :].astype(F32)
            lhs0[L + (s - 1) * PRE:L + s * PRE, :] = _ln(xs[16 - PRE:])

        @pl.loop(0, NP)
        def _(p):
            for c in w_copies(p):
                c.wait()

            @pl.when(p + AHEAD < NP)
            def _():
                for c in w_copies(p + AHEAD):
                    c.start()

            @pl.when(p + AHEAD == NP)
            def _():
                for c in f_copies:
                    c.start()

            for j in range(3):
                wt = stage[p, j]
                pbuf[p, j] = jax.lax.dot_general(lhs0[...], wt, NT, preferred_element_type=F32)
                wqkv[p, j] = wt.T

        acc = attend(lambda p, j: pbuf[p, j, 0:L, :])
        h_v[...] = finish(x_v[0:SEG, :].astype(F32), acc)
        mem = acc[:M]
        for c in f_copies:
            c.wait()

        mem = jax.lax.fori_loop(1, NA + 1, lambda s, m: step(s, m, True), mem, unroll=unroll)
        ra = pl.ds(0, NA * SEG)
        oc0 = pltpu.make_async_copy(o_v.at[ra, :], o_hbm.at[ra, :], sem_o.at[0])
        oc0.start()
        jax.lax.fori_loop(NA + 1, nsteps or NSEG, lambda s, m: step(s, m, False), mem, unroll=unroll)
        rb = pl.ds(NA * SEG, (NSEG - 1 - NA) * SEG)
        oc1 = pltpu.make_async_copy(o_v.at[rb, :], o_hbm.at[rb, :], sem_o.at[1])
        oc1.start()
        ffn_up()
        ffn_down(NSEG - 1)
        rc = pl.ds((NSEG - 1) * SEG, SEG)
        oc2 = pltpu.make_async_copy(o_v.at[rc, :], o_hbm.at[rc, :], sem_o.at[2])
        oc2.start()
        oc0.wait()
        oc1.wait()
        oc2.wait()

    return kernel


def _run(A_x, A_mem0, A_Wq, A_Wk, A_Wv, A_Wo, A_seg_len, B_x, B_w_gate, B_w_up, B_w_down, NA=40, **kw):
    B, S, D = A_x.shape
    _, H, Dh = A_Wq.shape
    M = A_mem0.shape[1]
    F = B_w_gate.shape[1]
    SEG = 32
    NP, PW = H // 2, 2 * Dh
    tr = lambda w: jnp.transpose(w, (1, 2, 0)).reshape(H * Dh, D)
    any_spec = pl.BlockSpec(memory_space=pl.ANY)
    out = pl.pallas_call(
        make_kernel(S, D, H, Dh, M, SEG, F, NA, **kw),
        out_shape=jax.ShapeDtypeStruct((S, D), A_x.dtype),
        in_specs=[any_spec, pl.BlockSpec(memory_space=pltpu.VMEM)] + [any_spec] * 7,
        out_specs=any_spec,
        scratch_shapes=[
            pltpu.VMEM((S, D), BF16), pltpu.VMEM((S, D), A_x.dtype),
            pltpu.VMEM((NP, 3, PW, D), BF16), pltpu.VMEM((NP, 3, D, PW), BF16),
            pltpu.VMEM((NP, PW, D), BF16),
            pltpu.VMEM((D, F), BF16), pltpu.VMEM((D, F), BF16), pltpu.VMEM((F, D), BF16),
            pltpu.VMEM((M + SEG + 8 * NA, D), F32), pltpu.VMEM((NP, 3, M + SEG + 8 * NA, PW), F32),
            pltpu.VMEM((SEG, D), F32), pltpu.VMEM((SEG, D), BF16), pltpu.VMEM((SEG, F), BF16),
            pltpu.SemaphoreType.DMA((NP, 4)), pltpu.SemaphoreType.DMA((1,)),
            pltpu.SemaphoreType.DMA((3,)), pltpu.SemaphoreType.DMA((3,)),
        ],
        compiler_params=pltpu.CompilerParams(vmem_limit_bytes=120 * 1024 * 1024),
    )(A_x.reshape(S, D), A_mem0.reshape(M, D), tr(A_Wq), tr(A_Wk), tr(A_Wv),
      A_Wo.reshape(H * Dh, D), B_w_gate, B_w_up, B_w_down)
    return out.reshape(B, S, D)


@functools.partial(jax.jit, static_argnames=("A_seg_len",))
def pallas_sequential_preLN__memory_aug_recurrent_mem_tr__swiglu_ffn__prompt_kernel(
    A_x, A_mem0, A_Wq, A_Wk, A_Wv, A_Wo, A_seg_len, B_x, B_w_gate, B_w_up, B_w_down,
):
    return _run(A_x, A_mem0, A_Wq, A_Wk, A_Wv, A_Wo, A_seg_len, B_x, B_w_gate, B_w_up, B_w_down)
```

```python
import functools

import jax
import jax.numpy as jnp
import jax.experimental.pallas as pl
import jax.experimental.pallas.tpu as pltpu

F32 = jnp.float32
BF16 = jnp.bfloat16
U32 = jnp.uint32
LANE = 128
PRE = 8
N_EARLY = 45


def _layernorm(x):
    d = x - jnp.mean(x, axis=-1, keepdims=True)
    v = jnp.mean(d * d, axis=-1, keepdims=True)
    return d * jax.lax.rsqrt(v + 1e-5)


def _dot(a, b):
    return jnp.dot(a, b, preferred_element_type=F32)


def _dot_nt(a, b):
    return jax.lax.dot_general(a, b, (((1,), (1,)), ((), ())), preferred_element_type=F32)


def _pack(w):
    return pltpu.bitcast(w, U32)


def _unpack(w):
    return pltpu.bitcast(w, BF16)


def _issue_order(n_pairs, lag_v=1, lag_o=4, tail="OOVOO"):
    lags = dict(P=0, S=0, V=lag_v, O=lag_o)
    ops = [(op, t - lags[op]) for t in range(n_pairs) for op in "PSVO" if t >= lags[op]]
    rest = {op: list(range(n_pairs - lag, n_pairs)) for op, lag in lags.items()}
    ops += [(op, rest[op].pop(0)) for op in tail]
    assert not any(rest.values())
    return ops


def _make_kernel(S, D, H, Dh, M, SEG, F):
    NP = H // 2
    PW = 2 * Dh
    L = M + SEG
    NSEG = S // SEG
    NA = N_EARLY
    R0 = L + PRE * NA
    assert PW == 3 * LANE and R0 % 16 == 0 and NA + 1 < NSEG
    scale = float(Dh) ** -0.5

    def kernel(x_hbm, mem0_ref, wq_hbm, wk_hbm, wv_hbm, wo_hbm, wg_hbm, wu_hbm, wd_hbm, o_hbm,
               x_v, xa_v, x0_v, o_v, lhs0, early, p0_v, h_v, hn_v, a_v,
               stage, wqkv, wo_s, wo_v, wg_v, wu_v, wd_v,
               sem_w, sem_f, sem_x, sem_o):

        def qkv_copies(p):
            r = pl.ds(pl.multiple_of(p * PW, PW), PW)
            return [pltpu.make_async_copy(w.at[r, :], stage.at[p, j], sem_w.at[p, j])
                    for j, w in enumerate((wk_hbm, wq_hbm, wv_hbm))]

        def x_copy(a, b, i):
            return pltpu.make_async_copy(x_hbm.at[pl.ds(a, b - a)], x_v.at[pl.ds(a, b - a)], sem_x.at[i])

        first_x = [
            pltpu.make_async_copy(x_hbm.at[0], x0_v, sem_x.at[0]),
            pltpu.make_async_copy(x_hbm.at[pl.ds(1, NA), pl.ds(SEG - PRE, PRE), :], xa_v, sem_x.at[1]),
        ]
        late = [pltpu.make_async_copy(w, v, sem_f.at[i])
                for i, (w, v) in enumerate(((wo_hbm, wo_s), (wg_hbm, wg_v), (wu_hbm, wu_v), (wd_hbm, wd_v)))]
        late.append(x_copy(1, NA + 1, 2))
        last_x = x_copy(NA + 1, NSEG, 3)
        for c in first_x + qkv_copies(0):
            c.start()

        row = jax.lax.broadcasted_iota(jnp.int32, (L, 2 * L), 0)
        col = jax.lax.broadcasted_iota(jnp.int32, (L, 2 * L), 1)
        head_a = col < L
        visible = (row < M) | (row >= jnp.where(head_a, col, col - L))
        lo_half = jax.lax.broadcasted_iota(jnp.int32, (L, LANE), 1) < Dh - LANE

        def blockdiag(t):
            t0, t1, t2 = (t[:, i * LANE:(i + 1) * LANE] for i in range(3))
            z = jnp.zeros((L, LANE), F32)
            a = jnp.concatenate([t0, jnp.where(lo_half, t1, 0.0), z], axis=1)
            b = jnp.concatenate([z, jnp.where(lo_half, 0.0, t1), t2], axis=1)
            return jnp.concatenate([a, b], axis=0).astype(BF16)

        def attention_probs(q, k):
            s = jnp.where(visible, _dot_nt(q, blockdiag(k)) * scale, -1e9)
            ma = jnp.max(jnp.where(head_a, s, -jnp.inf), axis=-1, keepdims=True)
            mb = jnp.max(jnp.where(head_a, -jnp.inf, s), axis=-1, keepdims=True)
            e = jnp.exp(s - jnp.where(head_a, ma, mb))
            la = jnp.sum(jnp.where(head_a, e, 0.0), axis=-1, keepdims=True)
            lb = jnp.sum(jnp.where(head_a, 0.0, e), axis=-1, keepdims=True)
            return e / jnp.where(head_a, la, lb)

        def ffn_up():
            hn = hn_v[...]
            hg = 0.5 * _dot(hn, wg_v[...])
            a_v[...] = ((hg + hg * jnp.tanh(hg)) * _dot(hn, wu_v[...])).astype(BF16)

        def ffn_down(s):
            o_v[s] = (h_v[...] + _dot(a_v[...], wd_v[...])).astype(o_v.dtype)

        def residual(xs, attn):
            h = xs + attn
            hn_v[...] = _layernorm(h).astype(BF16)
            return h

        def step(s, mem, early_rows=False):
            xn = _layernorm(x_v[s].astype(F32)[:SEG - PRE if early_rows else SEG])
            rows = jnp.concatenate([mem, xn], axis=0)
            if early_rows:
                rows = rows.astype(BF16)
                done = pl.ds(pl.multiple_of(L + (s - 1) * PRE, PRE), PRE)
            ffn_up()
            kqv, probs, mixed, acc = {}, {}, {}, None
            for op, p in _issue_order(NP):
                if op == "P":
                    y = _dot(rows, _unpack(wqkv[p]))
                    if early_rows:
                        y = jnp.concatenate([y, early[p, done, :]], axis=0)
                    kqv[p] = tuple(y[:, j * PW:(j + 1) * PW] for j in range(3))
                elif op == "S":
                    probs[p] = attention_probs(kqv[p][1], kqv[p][0])
                elif op == "V":
                    mixed[p] = _dot(probs[p], blockdiag(kqv[p][2]))
                else:
                    y = _dot(mixed[p], _unpack(wo_v[p]))
                    acc = y if acc is None else acc + y
            h = residual(x_v[s].astype(F32), acc[M:])
            ffn_down(s - 1)
            h_v[...] = h
            return acc[:M]

        for c in first_x:
            c.wait()
        for c in qkv_copies(1):
            c.start()
        for c in late:
            c.start(priority=1)
        lhs0[...] = _pack(jnp.concatenate(
            [mem0_ref[...].astype(F32), _layernorm(x0_v[...].astype(F32)),
             _layernorm(xa_v[...].astype(F32).reshape(NA * PRE, D))], axis=0).astype(BF16))

        @pl.loop(0, NP)
        def _(p):
            for c in qkv_copies(p):
                c.wait()

            @pl.when(p + 2 < NP)
            def _():
                for c in qkv_copies(p + 2):
                    c.start()

            def project(j, c0=0, c1=PW):
                wt = stage[p, j, c0:c1, :]
                wqkv[p, :, j * PW + c0:j * PW + c1] = _pack(wt.T)
                y = _dot_nt(_unpack(lhs0[...]), wt)
                early[p, :, j * PW + c0:j * PW + c1] = y
                return y[:L]

            k = project(0)
            q = project(1)
            project(2, 0, LANE)
            p0_v[p] = attention_probs(q, k)
            project(2, LANE, PW)

        late[0].wait()
        mixed, acc = {}, None
        for t in range(NP + 1):
            if t < NP:
                mixed[t] = _dot(p0_v[t], blockdiag(early[t, 0:L, 2 * PW:]))
            if t >= 1:
                wo = wo_s[(t - 1) * PW:t * PW, :]
                wo_v[t - 1] = _pack(wo)
                y = _dot(mixed[t - 1], wo)
                acc = y if acc is None else acc + y
        h_v[...] = residual(x0_v[...].astype(F32), acc[M:])
        last_x.start()
        for c in late[1:]:
            c.wait()

        bounds = (0, NA, NSEG - 1, NSEG)
        out_copies = [pltpu.make_async_copy(o_v.at[pl.ds(a, b - a)], o_hbm.at[pl.ds(a, b - a)], sem_o.at[i])
                      for i, (a, b) in enumerate(zip(bounds[:-1], bounds[1:]))]
        mem = jax.lax.fori_loop(1, NA + 1, functools.partial(step, early_rows=True), acc[:M], unroll=3)
        last_x.wait()
        out_copies[0].start()
        jax.lax.fori_loop(NA + 1, NSEG, step, mem, unroll=2)
        out_copies[1].start()
        ffn_up()
        ffn_down(NSEG - 1)
        out_copies[2].start()
        for c in out_copies:
            c.wait()

    scratch = [
        pltpu.VMEM((NSEG, SEG, D), BF16), pltpu.VMEM((NA, PRE, D), BF16), pltpu.VMEM((SEG, D), BF16),
        pltpu.VMEM((NSEG, SEG, D), BF16),
        pltpu.VMEM((R0 // 2, D), U32), pltpu.VMEM((NP, R0, 3 * PW), F32), pltpu.VMEM((NP, L, 2 * L), F32),
        pltpu.VMEM((SEG, D), F32), pltpu.VMEM((SEG, D), BF16), pltpu.VMEM((SEG, F), BF16),
        pltpu.VMEM((NP, 3, PW, D), BF16), pltpu.VMEM((NP, D // 2, 3 * PW), U32),
        pltpu.VMEM((H * Dh, D), BF16), pltpu.VMEM((NP, PW // 2, D), U32),
        pltpu.VMEM((D, F), BF16), pltpu.VMEM((D, F), BF16), pltpu.VMEM((F, D), BF16),
        pltpu.SemaphoreType.DMA((NP, 3)), pltpu.SemaphoreType.DMA((4,)),
        pltpu.SemaphoreType.DMA((4,)), pltpu.SemaphoreType.DMA((3,)),
    ]
    return kernel, scratch


@functools.partial(jax.jit, static_argnames=("A_seg_len",))
def pallas_sequential_preLN__memory_aug_recurrent_mem_tr__swiglu_ffn__prompt_kernel(
    A_x: jax.Array,
    A_mem0: jax.Array,
    A_Wq: jax.Array,
    A_Wk: jax.Array,
    A_Wv: jax.Array,
    A_Wo: jax.Array,
    A_seg_len: int,
    B_x: jax.Array,
    B_w_gate: jax.Array,
    B_w_up: jax.Array,
    B_w_down: jax.Array,
):
    B, S, D = A_x.shape
    _, H, Dh = A_Wq.shape
    M = A_mem0.shape[1]
    F = B_w_gate.shape[1]
    SEG = int(A_seg_len)
    assert B == 1

    def rows_by_head(w):
        return jnp.transpose(w, (1, 2, 0)).reshape(H * Dh, D)

    hbm = pl.BlockSpec(memory_space=pl.ANY)
    kernel, scratch = _make_kernel(S, D, H, Dh, M, SEG, F)
    out = pl.pallas_call(
        kernel,
        out_shape=jax.ShapeDtypeStruct((S // SEG, SEG, D), A_x.dtype),
        in_specs=[hbm, pl.BlockSpec(memory_space=pltpu.VMEM)] + [hbm] * 7,
        out_specs=hbm,
        scratch_shapes=scratch,
        compiler_params=pltpu.CompilerParams(vmem_limit_bytes=120 * 1024 * 1024),
    )(A_x.reshape(S // SEG, SEG, D), A_mem0.reshape(M, D), rows_by_head(A_Wq), rows_by_head(A_Wk),
      rows_by_head(A_Wv), A_Wo.reshape(H * Dh, D), B_w_gate, B_w_up, B_w_down)
    return out.reshape(B, S, D)
```

```python
import functools

import jax
import jax.numpy as jnp
import jax.experimental.pallas as pl
import jax.experimental.pallas.tpu as pltpu

F32 = jnp.float32
BF16 = jnp.bfloat16
U32 = jnp.uint32
LANE = 128
PRE = 8
N_EARLY = 45


def _layernorm(x):
    d = x - jnp.mean(x, axis=-1, keepdims=True)
    v = jnp.mean(d * d, axis=-1, keepdims=True)
    return d * jax.lax.rsqrt(v + 1e-5)


def _dot(a, b):
    return jnp.dot(a, b, preferred_element_type=F32)


def _dot_nt(a, b):
    return jax.lax.dot_general(a, b, (((1,), (1,)), ((), ())), preferred_element_type=F32)


def _pack(w):
    return pltpu.bitcast(w, U32)


def _unpack(w):
    return pltpu.bitcast(w, BF16)


def _issue_order(n_pairs, lag_v=1, lag_o=4, tail="OOVOO"):
    lags = dict(P=0, S=0, V=lag_v, O=lag_o)
    ops = [(op, t - lags[op]) for t in range(n_pairs) for op in "PSVO" if t >= lags[op]]
    rest = {op: list(range(n_pairs - lag, n_pairs)) for op, lag in lags.items()}
    ops += [(op, rest[op].pop(0)) for op in tail]
    assert not any(rest.values())
    return ops


def _make_kernel(S, D, H, Dh, M, SEG, F):
    NP = H // 2
    PW = 2 * Dh
    L = M + SEG
    NSEG = S // SEG
    NA = N_EARLY
    R0 = L + PRE * NA
    assert PW == 3 * LANE and R0 % 16 == 0 and NA + 1 < NSEG
    scale = float(Dh) ** -0.5

    def kernel(x_hbm, mem_hbm, wq_hbm, wk_hbm, wv_hbm, wo_hbm, wg_hbm, wu_hbm, wd_hbm, o_hbm,
               x_v, xa_v, x0_v, mem_v, o_v, lhs0, early, p0_v, h_v, hn_v, a_v,
               stage, wqkv, wo_s, wo_v, wg_v, wu_v, wd_v,
               sem_w, sem_wo, sem_late, sem_x, sem_o):

        def qkv_copies(p):
            r = pl.ds(pl.multiple_of(p * PW, PW), PW)
            return [pltpu.make_async_copy(w.at[r, :], stage.at[p, j], sem_w.at[p % 3])
                    for j, w in enumerate((wk_hbm, wq_hbm, wv_hbm))]

        def x_copy(a, b, sem):
            return pltpu.make_async_copy(x_hbm.at[pl.ds(a, b - a)], x_v.at[pl.ds(a, b - a)], sem)

        first_x = [
            pltpu.make_async_copy(mem_hbm, mem_v, sem_x),
            pltpu.make_async_copy(x_hbm.at[0], x0_v, sem_x),
            pltpu.make_async_copy(x_hbm.at[pl.ds(1, NA), pl.ds(SEG - PRE, PRE), :], xa_v, sem_x),
        ]
        wo_copy = pltpu.make_async_copy(wo_hbm, wo_s, sem_wo)
        late = [pltpu.make_async_copy(w, v, sem_late) for w, v in ((wg_hbm, wg_v), (wu_hbm, wu_v), (wd_hbm, wd_v))]
        late.append(x_copy(1, NA + 1, sem_late))
        last_x = x_copy(NA + 1, NSEG, sem_x)
        for c in first_x + qkv_copies(0):
            c.start()

        row = jax.lax.broadcasted_iota(jnp.int32, (L, 2 * L), 0)
        col = jax.lax.broadcasted_iota(jnp.int32, (L, 2 * L), 1)
        head_a = col < L
        visible = (row < M) | (row >= jnp.where(head_a, col, col - L))
        lo_half = jax.lax.broadcasted_iota(jnp.int32, (L, LANE), 1) < Dh - LANE

        def blockdiag(t):
            t0, t1, t2 = (t[:, i * LANE:(i + 1) * LANE] for i in range(3))
            z = jnp.zeros((L, LANE), F32)
            a = jnp.concatenate([t0, jnp.where(lo_half, t1, 0.0), z], axis=1)
            b = jnp.concatenate([z, jnp.where(lo_half, 0.0, t1), t2], axis=1)
            return jnp.concatenate([a, b], axis=0).astype(BF16)

        def attention_probs(q, k):
            s = jnp.where(visible, _dot_nt(q, blockdiag(k)) * scale, -1e9)
            ma = jnp.max(jnp.where(head_a, s, -jnp.inf), axis=-1, keepdims=True)
            mb = jnp.max(jnp.where(head_a, -jnp.inf, s), axis=-1, keepdims=True)
            e = jnp.exp(s - jnp.where(head_a, ma, mb))
            la = jnp.sum(jnp.where(head_a, e, 0.0), axis=-1, keepdims=True)
            lb = jnp.sum(jnp.where(head_a, 0.0, e), axis=-1, keepdims=True)
            return e / jnp.where(head_a, la, lb)

        def ffn_up():
            hn = hn_v[...]
            hg = 0.5 * _dot(hn, wg_v[...])
            a_v[...] = ((hg + hg * jnp.tanh(hg)) * _dot(hn, wu_v[...])).astype(BF16)

        def ffn_down(s):
            o_v[s] = (h_v[...] + _dot(a_v[...], wd_v[...])).astype(o_v.dtype)

        def residual(xs, attn):
            h = xs + attn
            hn_v[...] = _layernorm(h).astype(BF16)
            return h

        def step(s, mem, early_rows=False):
            xn = _layernorm(x_v[s].astype(F32)[:SEG - PRE if early_rows else SEG])
            rows = jnp.concatenate([mem, xn], axis=0)
            if early_rows:
                rows = rows.astype(BF16)
                done = pl.ds(pl.multiple_of(L + (s - 1) * PRE, PRE), PRE)
            ffn_up()
            kqv, probs, mixed, acc = {}, {}, {}, None
            for op, p in _issue_order(NP):
                if op == "P":
                    y = _dot(rows, _unpack(wqkv[p]))
                    if early_rows:
                        y = jnp.concatenate([y, early[p, done, :]], axis=0)
                    kqv[p] = tuple(y[:, j * PW:(j + 1) * PW] for j in range(3))
                elif op == "S":
                    probs[p] = attention_probs(kqv[p][1], kqv[p][0])
                elif op == "V":
                    mixed[p] = _dot(probs[p], blockdiag(kqv[p][2]))
                else:
                    y = _dot(mixed[p], _unpack(wo_v[p]))
                    acc = y if acc is None else acc + y
            h = residual(x_v[s].astype(F32), acc[M:])
            ffn_down(s - 1)
            h_v[...] = h
            return acc[:M]

        for c in first_x:
            c.wait()
        for c in qkv_copies(1):
            c.start()
        for c in [wo_copy] + late:
            c.start(priority=1)
        lhs0[...] = _pack(jnp.concatenate(
            [mem_v[...].astype(F32), _layernorm(x0_v[...].astype(F32)),
             _layernorm(xa_v[...].astype(F32).reshape(NA * PRE, D))], axis=0).astype(BF16))

        @pl.loop(0, NP)
        def _(p):
            for c in qkv_copies(p):
                c.wait()

            @pl.when(p + 2 < NP)
            def _():
                for c in qkv_copies(p + 2):
                    c.start()

            def project(j, c0=0, c1=PW):
                wt = stage[p, j, c0:c1, :]
                wqkv[p, :, j * PW + c0:j * PW + c1] = _pack(wt.T)
                y = _dot_nt(_unpack(lhs0[...]), wt)
                early[p, :, j * PW + c0:j * PW + c1] = y
                return y[:L]

            k = project(0)
            q = project(1)
            project(2, 0, LANE)
            p0_v[p] = attention_probs(q, k)
            project(2, LANE, PW)

        wo_copy.wait()
        mixed, acc = {}, None
        for t in range(NP + 1):
            if t < NP:
                mixed[t] = _dot(p0_v[t], blockdiag(early[t, 0:L, 2 * PW:]))
            if t >= 1:
                wo = wo_s[(t - 1) * PW:t * PW, :]
                wo_v[t - 1] = _pack(wo)
                y = _dot(mixed[t - 1], wo)
                acc = y if acc is None else acc + y
        h_v[...] = residual(x0_v[...].astype(F32), acc[M:])
        last_x.start()
        for c in late:
            c.wait()

        bounds = (0, NA, NSEG - 1, NSEG)
        out_copies = [pltpu.make_async_copy(o_v.at[pl.ds(a, b - a)], o_hbm.at[pl.ds(a, b - a)], sem_o)
                      for a, b in zip(bounds[:-1], bounds[1:])]
        mem = jax.lax.fori_loop(1, NA + 1, functools.partial(step, early_rows=True), acc[:M], unroll=3)
        last_x.wait()
        out_copies[0].start()
        jax.lax.fori_loop(NA + 1, NSEG, step, mem, unroll=2)
        out_copies[1].start()
        ffn_up()
        ffn_down(NSEG - 1)
        out_copies[2].start()
        for c in out_copies:
            c.wait()

    scratch = [
        pltpu.VMEM((NSEG, SEG, D), BF16), pltpu.VMEM((NA, PRE, D), BF16), pltpu.VMEM((SEG, D), BF16),
        pltpu.VMEM((M, D), BF16), pltpu.VMEM((NSEG, SEG, D), BF16),
        pltpu.VMEM((R0 // 2, D), U32), pltpu.VMEM((NP, R0, 3 * PW), F32), pltpu.VMEM((NP, L, 2 * L), F32),
        pltpu.VMEM((SEG, D), F32), pltpu.VMEM((SEG, D), BF16), pltpu.VMEM((SEG, F), BF16),
        pltpu.VMEM((NP, 3, PW, D), BF16), pltpu.VMEM((NP, D // 2, 3 * PW), U32),
        pltpu.VMEM((H * Dh, D), BF16), pltpu.VMEM((NP, PW // 2, D), U32),
        pltpu.VMEM((D, F), BF16), pltpu.VMEM((D, F), BF16), pltpu.VMEM((F, D), BF16),
        pltpu.SemaphoreType.DMA((3,)), pltpu.SemaphoreType.DMA, pltpu.SemaphoreType.DMA,
        pltpu.SemaphoreType.DMA, pltpu.SemaphoreType.DMA,
    ]
    return kernel, scratch


@functools.partial(jax.jit, static_argnames=("A_seg_len",))
def pallas_sequential_preLN__memory_aug_recurrent_mem_tr__swiglu_ffn__prompt_kernel(
    A_x: jax.Array,
    A_mem0: jax.Array,
    A_Wq: jax.Array,
    A_Wk: jax.Array,
    A_Wv: jax.Array,
    A_Wo: jax.Array,
    A_seg_len: int,
    B_x: jax.Array,
    B_w_gate: jax.Array,
    B_w_up: jax.Array,
    B_w_down: jax.Array,
):
    B, S, D = A_x.shape
    _, H, Dh = A_Wq.shape
    M = A_mem0.shape[1]
    F = B_w_gate.shape[1]
    SEG = int(A_seg_len)
    assert B == 1

    def rows_by_head(w):
        return jnp.transpose(w, (1, 2, 0)).reshape(H * Dh, D)

    hbm = pl.BlockSpec(memory_space=pl.ANY)
    kernel, scratch = _make_kernel(S, D, H, Dh, M, SEG, F)
    out = pl.pallas_call(
        kernel,
        out_shape=jax.ShapeDtypeStruct((S // SEG, SEG, D), A_x.dtype),
        in_specs=[hbm] * 9,
        out_specs=hbm,
        scratch_shapes=scratch,
        compiler_params=pltpu.CompilerParams(vmem_limit_bytes=120 * 1024 * 1024),
    )(A_x.reshape(S // SEG, SEG, D), A_mem0.reshape(M, D), rows_by_head(A_Wq), rows_by_head(A_Wk),
      rows_by_head(A_Wv), A_Wo.reshape(H * Dh, D), B_w_gate, B_w_up, B_w_down)
    return out.reshape(B, S, D)
```

```python
import functools

import jax
import jax.numpy as jnp
import jax.experimental.pallas as pl
import jax.experimental.pallas.tpu as pltpu

F32 = jnp.float32
BF16 = jnp.bfloat16
U32 = jnp.uint32
LANE = 128
PRE = 8
N_EARLY = 45


def _layernorm(x):
    d = x - jnp.mean(x, axis=-1, keepdims=True)
    v = jnp.mean(d * d, axis=-1, keepdims=True)
    return d * jax.lax.rsqrt(v + 1e-5)


def _dot(a, b):
    return jnp.dot(a, b, preferred_element_type=F32)


def _dot_nt(a, b):
    return jax.lax.dot_general(a, b, (((1,), (1,)), ((), ())), preferred_element_type=F32)


def _pack(w):
    return pltpu.bitcast(w, U32)


def _unpack(w):
    return pltpu.bitcast(w, BF16)


def _issue_order(n_pairs, lag_v=1, lag_o=4, tail="OOVOO"):
    lags = dict(P=0, S=0, V=lag_v, O=lag_o)
    ops = [(op, t - lags[op]) for t in range(n_pairs) for op in "PSVO" if t >= lags[op]]
    rest = {op: list(range(n_pairs - lag, n_pairs)) for op, lag in lags.items()}
    ops += [(op, rest[op].pop(0)) for op in tail]
    assert not any(rest.values())
    return ops


def _make_kernel(S, D, H, Dh, M, SEG, F):
    NP = H // 2
    PW = 2 * Dh
    L = M + SEG
    NSEG = S // SEG
    NA = N_EARLY
    R0 = L + PRE * NA
    assert PW == 3 * LANE and R0 % 16 == 0 and NA + 1 < NSEG
    scale = float(Dh) ** -0.5

    def kernel(x_hbm, mem_hbm, wq_hbm, wk_hbm, wv_hbm, wo_hbm, wg_hbm, wu_hbm, wd_hbm, o_hbm,
               x_v, xa_v, x0_v, mem_v, o_v, lhs0, early, p0_v, h_v, hn_v, a_v,
               stage, wqkv, wo_s, wo_v, wg_v, wu_v, wd_v,
               sem_w, sem_wo, sem_late, sem_x, sem_o):

        def qkv_copies(p):
            r = pl.ds(pl.multiple_of(p * PW, PW), PW)
            return [pltpu.make_async_copy(w.at[r, :], stage.at[p, pl.ds(j * PW, PW), :], sem_w.at[p % 3])
                    for j, w in enumerate((wk_hbm, wq_hbm, wv_hbm))]

        def x_copy(a, b, sem):
            return pltpu.make_async_copy(x_hbm.at[pl.ds(a, b - a)], x_v.at[pl.ds(a, b - a)], sem)

        first_x = [
            pltpu.make_async_copy(mem_hbm, mem_v, sem_x),
            pltpu.make_async_copy(x_hbm.at[0], x0_v, sem_x),
            pltpu.make_async_copy(x_hbm.at[pl.ds(1, NA), pl.ds(SEG - PRE, PRE), :], xa_v, sem_x),
        ]
        wo_copy = pltpu.make_async_copy(wo_hbm, wo_s, sem_wo)
        late = [pltpu.make_async_copy(w, v, sem_late) for w, v in ((wg_hbm, wg_v), (wu_hbm, wu_v), (wd_hbm, wd_v))]
        late.append(x_copy(1, NA + 1, sem_late))
        last_x = x_copy(NA + 1, NSEG, sem_x)
        for c in first_x + qkv_copies(0):
            c.start()

        row = jax.lax.broadcasted_iota(jnp.int32, (L, 2 * L), 0)
        col = jax.lax.broadcasted_iota(jnp.int32, (L, 2 * L), 1)
        head_a = col < L
        visible = (row < M) | (row >= jnp.where(head_a, col, col - L))
        lo_half = jax.lax.broadcasted_iota(jnp.int32, (L, LANE), 1) < Dh - LANE

        def blockdiag(t):
            t0, t1, t2 = (t[:, i * LANE:(i + 1) * LANE] for i in range(3))
            z = jnp.zeros((L, LANE), F32)
            a = jnp.concatenate([t0, jnp.where(lo_half, t1, 0.0), z], axis=1)
            b = jnp.concatenate([z, jnp.where(lo_half, 0.0, t1), t2], axis=1)
            return jnp.concatenate([a, b], axis=0).astype(BF16)

        def attention_probs(q, k):
            s = jnp.where(visible, _dot_nt(q, blockdiag(k)) * scale, -1e9)
            ma = jnp.max(jnp.where(head_a, s, -jnp.inf), axis=-1, keepdims=True)
            mb = jnp.max(jnp.where(head_a, -jnp.inf, s), axis=-1, keepdims=True)
            e = jnp.exp(s - jnp.where(head_a, ma, mb))
            la = jnp.sum(jnp.where(head_a, e, 0.0), axis=-1, keepdims=True)
            lb = jnp.sum(jnp.where(head_a, 0.0, e), axis=-1, keepdims=True)
            return e / jnp.where(head_a, la, lb)

        def ffn_up():
            hn = hn_v[...]
            hg = 0.5 * _dot(hn, wg_v[...])
            a_v[...] = ((hg + hg * jnp.tanh(hg)) * _dot(hn, wu_v[...])).astype(BF16)

        def ffn_down(s):
            o_v[s] = (h_v[...] + _dot(a_v[...], wd_v[...])).astype(o_v.dtype)

        def residual(xs, attn):
            h = xs + attn
            hn_v[...] = _layernorm(h).astype(BF16)
            return h

        def step(s, mem, early_rows=False):
            xn = _layernorm(x_v[s].astype(F32)[:SEG - PRE if early_rows else SEG])
            rows = jnp.concatenate([mem, xn], axis=0)
            if early_rows:
                rows = rows.astype(BF16)
                done = pl.ds(pl.multiple_of(L + (s - 1) * PRE, PRE), PRE)
            ffn_up()
            kqv, probs, mixed, acc = {}, {}, {}, None
            for op, p in _issue_order(NP):
                if op == "P":
                    y = _dot(rows, _unpack(wqkv[p]))
                    if early_rows:
                        y = jnp.concatenate([y, early[p, done, :]], axis=0)
                    kqv[p] = tuple(y[:, j * PW:(j + 1) * PW] for j in range(3))
                elif op == "S":
                    probs[p] = attention_probs(kqv[p][1], kqv[p][0])
                elif op == "V":
                    mixed[p] = _dot(probs[p], blockdiag(kqv[p][2]))
                else:
                    y = _dot(mixed[p], _unpack(wo_v[p]))
                    acc = y if acc is None else acc + y
            h = residual(x_v[s].astype(F32), acc[M:])
            ffn_down(s - 1)
            h_v[...] = h
            return acc[:M]

        for c in first_x:
            c.wait()
        for c in qkv_copies(1):
            c.start()
        for c in [wo_copy] + late:
            c.start(priority=1)
        lhs0[...] = _pack(jnp.concatenate(
            [mem_v[...].astype(F32), _layernorm(x0_v[...].astype(F32)),
             _layernorm(xa_v[...].astype(F32).reshape(NA * PRE, D))], axis=0).astype(BF16))

        @pl.loop(0, NP)
        def _(p):
            for c in qkv_copies(p):
                c.wait()

            @pl.when(p + 2 < NP)
            def _():
                for c in qkv_copies(p + 2):
                    c.start()

            def project(c0, c1, r0=0, r1=R0):
                wt = stage[p, c0:c1, :]
                if r0 == 0:
                    wqkv[p, :, c0:c1] = _pack(wt.T)
                y = _dot_nt(_unpack(lhs0[r0 // 2:r1 // 2, :]), wt)
                early[p, r0:r1, c0:c1] = y
                return y[:L]

            y = jnp.concatenate([project(0, LANE), project(LANE, 5 * LANE),
                                 project(5 * LANE, 3 * PW, 0, LANE)], axis=1)
            p0_v[p] = attention_probs(y[:, PW:2 * PW], y[:, :PW])
            project(5 * LANE, 3 * PW, LANE, R0)

        wo_copy.wait()
        mixed, acc = {}, None
        for t in range(NP + 1):
            if t < NP:
                mixed[t] = _dot(p0_v[t], blockdiag(early[t, 0:L, 2 * PW:]))
            if t >= 1:
                wo = wo_s[(t - 1) * PW:t * PW, :]
                wo_v[t - 1] = _pack(wo)
                y = _dot(mixed[t - 1], wo)
                acc = y if acc is None else acc + y
        h_v[...] = residual(x0_v[...].astype(F32), acc[M:])
        last_x.start()
        for c in late:
            c.wait()

        bounds = (0, NA, NSEG - 1, NSEG)
        out_copies = [pltpu.make_async_copy(o_v.at[pl.ds(a, b - a)], o_hbm.at[pl.ds(a, b - a)], sem_o)
                      for a, b in zip(bounds[:-1], bounds[1:])]
        mem = jax.lax.fori_loop(1, NA + 1, functools.partial(step, early_rows=True), acc[:M], unroll=3)
        last_x.wait()
        out_copies[0].start()
        jax.lax.fori_loop(NA + 1, NSEG, step, mem, unroll=2)
        out_copies[1].start()
        ffn_up()
        ffn_down(NSEG - 1)
        out_copies[2].start()
        for c in out_copies:
            c.wait()

    scratch = [
        pltpu.VMEM((NSEG, SEG, D), BF16), pltpu.VMEM((NA, PRE, D), BF16), pltpu.VMEM((SEG, D), BF16),
        pltpu.VMEM((M, D), BF16), pltpu.VMEM((NSEG, SEG, D), BF16),
        pltpu.VMEM((R0 // 2, D), U32), pltpu.VMEM((NP, R0, 3 * PW), F32), pltpu.VMEM((NP, L, 2 * L), F32),
        pltpu.VMEM((SEG, D), F32), pltpu.VMEM((SEG, D), BF16), pltpu.VMEM((SEG, F), BF16),
        pltpu.VMEM((NP, 3 * PW, D), BF16), pltpu.VMEM((NP, D // 2, 3 * PW), U32),
        pltpu.VMEM((H * Dh, D), BF16), pltpu.VMEM((NP, PW // 2, D), U32),
        pltpu.VMEM((D, F), BF16), pltpu.VMEM((D, F), BF16), pltpu.VMEM((F, D), BF16),
        pltpu.SemaphoreType.DMA((3,)), pltpu.SemaphoreType.DMA, pltpu.SemaphoreType.DMA,
        pltpu.SemaphoreType.DMA, pltpu.SemaphoreType.DMA,
    ]
    return kernel, scratch


@functools.partial(jax.jit, static_argnames=("A_seg_len",))
def pallas_sequential_preLN__memory_aug_recurrent_mem_tr__swiglu_ffn__prompt_kernel(
    A_x: jax.Array,
    A_mem0: jax.Array,
    A_Wq: jax.Array,
    A_Wk: jax.Array,
    A_Wv: jax.Array,
    A_Wo: jax.Array,
    A_seg_len: int,
    B_x: jax.Array,
    B_w_gate: jax.Array,
    B_w_up: jax.Array,
    B_w_down: jax.Array,
):
    B, S, D = A_x.shape
    _, H, Dh = A_Wq.shape
    M = A_mem0.shape[1]
    F = B_w_gate.shape[1]
    SEG = int(A_seg_len)
    assert B == 1

    def rows_by_head(w):
        return jnp.transpose(w, (1, 2, 0)).reshape(H * Dh, D)

    hbm = pl.BlockSpec(memory_space=pl.ANY)
    kernel, scratch = _make_kernel(S, D, H, Dh, M, SEG, F)
    out = pl.pallas_call(
        kernel,
        out_shape=jax.ShapeDtypeStruct((S // SEG, SEG, D), A_x.dtype),
        in_specs=[hbm] * 9,
        out_specs=hbm,
        scratch_shapes=scratch,
        compiler_params=pltpu.CompilerParams(vmem_limit_bytes=120 * 1024 * 1024),
    )(A_x.reshape(S // SEG, SEG, D), A_mem0.reshape(M, D), rows_by_head(A_Wq), rows_by_head(A_Wk),
      rows_by_head(A_Wv), A_Wo.reshape(H * Dh, D), B_w_gate, B_w_up, B_w_down)
    return out.reshape(B, S, D)
```
